```python
import os as _os
_os.environ.setdefault("JAX_PLATFORMS", "cpu")
import jax
import jax.numpy as jnp

def _softmax(x, axis=-1):
    return jax.nn.softmax(x, axis=axis)
def _gelu(x):
    return jax.nn.gelu(x, approximate=True)
def _silu(x):
    return jax.nn.silu(x)
def _sigmoid(x):
    return jax.nn.sigmoid(x)
def _layernorm(x, axis=-1, eps=1e-5):
    m = jnp.mean(x, axis=axis, keepdims=True)
    v = jnp.var(x, axis=axis, keepdims=True)
    return (x - m) / jnp.sqrt(v + eps)
def _scatter_add(tgt, idx, src, axis=0):
    return tgt.at[idx].add(src)
def _segment_sum(src, seg, n):
    return jax.ops.segment_sum(src, seg, n)
class _Rng:
    def __init__(self, key):
        self._k = key
    def _next(self):
        self._k, sub = jax.random.split(self._k)
        return sub
    def normal(self, shape):
        return jax.random.normal(self._next(), shape, dtype=jnp.bfloat16)
    def randint(self, lo, hi, shape):
        return jax.random.randint(self._next(), shape, lo, hi, dtype=jnp.int32)
    def uniform(self, shape, lo=0.0, hi=1.0):
        return jax.random.uniform(self._next(), shape, jnp.bfloat16, lo, hi)
    def permutation(self, n):
        return jax.random.permutation(self._next(), n)


kernel_name = 'standalone__channel_attn_cbam__vision'

def setup_inputs():
    _rng = _Rng(jax.random.key(int.from_bytes(__import__("os").urandom(4), "little")))
    _w = (lambda a: (lambda t: t.astype(jnp.bfloat16) if jnp.issubdtype(t.dtype, jnp.floating) else t)(jnp.asarray(a)))
    H = W = 224
    C = 192
    r = max(C // 4, 1)
    return {
        "x": _w((lambda *s: _rng.normal(s) * 0.2)(1, H, W, C) + (lambda *s: _rng.normal(s) * 0.2)(1, 1, 1, C) * 2.0),
        "w1": _w((lambda *s: _rng.normal(s) * 0.2)(C, r)),
        "w2": _w((lambda *s: _rng.normal(s) * 0.2)(r, C)),
    }

def reference(x, w1, w2):
    B, H, W, C = x.shape
    xf = x.reshape(B, H * W, C)
    gap = jnp.mean(xf, 1)
    gmp = jnp.amax(xf, 1)
    h_a = gap @ w1
    h_a = h_a * (lambda x, dt: x.astype(dt))(h_a > 0, h_a.dtype)
    h_m = gmp @ w1
    h_m = h_m * (lambda x, dt: x.astype(dt))(h_m > 0, h_m.dtype)
    scale = _sigmoid(h_a @ w2 + h_m @ w2)
    return x * scale[:, None, None, :]
```

```python
import jax
import jax.numpy as jnp
import jax.experimental.pallas as pl
import jax.experimental.pallas.tpu as pltpu

S = 8
KR = 16
RSPLIT = 2
D = 5
CB = 32
KW = 16
TAIL = 3


@jax.jit
def pallas_standalone__channel_attn_cbam__vision_kernel(
    x: jax.Array,
    w1: jax.Array,
    w2: jax.Array,
):
    B, H, W, C = x.shape
    R = w1.shape[1]
    Hs = H // S
    shp = (S, Hs, C, W)
    inv_n = 1.0 / (H * W)
    SP = S // RSPLIT

    def kernel(x_hbm, w1t_hbm, w2_hbm, o_hbm, buf, w1t_v, w2_v, sum_ref, max_ref, scale_ref, sems):
        wsem = sems.at[D]

        def start_group(t, slot, c0=0, c1=C):
            for cb in range(c0 // KR, c1 // KR):
                for p in range(RSPLIT):
                    idx = (pl.ds(p * SP, SP), pl.ds(t, 1), pl.ds(cb * KR, KR))
                    pltpu.make_async_copy(x_hbm.at[idx], buf.at[idx], sems.at[slot]).start(
                        priority=p % 2)

        def wait_group(t, slot, c0=0, c1=C):
            idx = (slice(None), pl.ds(t, 1), pl.ds(c0, c1 - c0))
            pltpu.make_async_copy(x_hbm.at[idx], buf.at[idx], sems.at[slot]).wait()

        def accumulate(t, c0=0, c1=C):
            for cb in range(c0 // CB, c1 // CB):
                rows = pl.ds(cb * CB, CB)
                sa = ma = None
                for s in range(S):
                    v = buf[s, t, rows, :].astype(jnp.float32)
                    sa = v if s == 0 else sa + v
                    ma = v if s == 0 else jnp.maximum(ma, v)
                sum_ref[rows, :] = sum_ref[rows, :] + sa
                max_ref[rows, :] = jnp.maximum(max_ref[rows, :], ma)

        nfull = Hs - 1
        tail = [(Hs - 1, i * (C // TAIL), (i + 1) * (C // TAIL)) for i in range(TAIL)]
        for t in range(D):
            start_group(t, t)
        cw1 = pltpu.make_async_copy(w1t_hbm, w1t_v, wsem)
        cw2 = pltpu.make_async_copy(w2_hbm, w2_v, wsem)
        cw1.start()
        cw2.start()
        sum_ref[...] = jnp.zeros(sum_ref.shape, jnp.float32)
        max_ref[...] = jnp.full(max_ref.shape, -jnp.inf, jnp.float32)

        def body(t, carry):
            slot = jax.lax.rem(t, D)
            wait_group(t, slot)
            start_group(t + D, slot)
            accumulate(t)
            return carry

        jax.lax.fori_loop(0, nfull - D, body, 0)
        rest = [(t, 0, C) for t in range(nfull - D, nfull)] + tail
        g0 = nfull - D
        for i, (t, c0, c1) in enumerate(rest):
            g = g0 + i
            wait_group(t, g % D, c0, c1)
            if i + D < len(rest):
                t2, c02, c12 = rest[i + D]
                start_group(t2, g % D, c02, c12)
            if i == 0:
                cw1.wait()
                cw2.wait()
            accumulate(t, c0, c1)

        gap = (jnp.sum(sum_ref[...], axis=1, keepdims=True) * inv_n).astype(jnp.bfloat16)
        gmp = jnp.max(max_ref[...], axis=1, keepdims=True).astype(jnp.bfloat16)
        lane = jax.lax.broadcasted_iota(jnp.int32, (C, 128), 1)
        P = jnp.where(lane < 64, jnp.broadcast_to(gap.astype(jnp.float32), (C, 128)),
                      jnp.broadcast_to(gmp.astype(jnp.float32), (C, 128))).astype(jnp.bfloat16)
        h = jnp.dot(w1t_v[...], P, preferred_element_type=jnp.float32)
        h = jnp.maximum(h.astype(jnp.bfloat16).astype(jnp.float32), 0.0).astype(jnp.bfloat16)
        z = jax.lax.dot_general(w2_v[...], h, (((0,), (0,)), ((), ())),
                                preferred_element_type=jnp.float32)
        z = z.astype(jnp.bfloat16).astype(jnp.float32)
        zz = (z[:, 0:1] + z[:, 64:65]).astype(jnp.bfloat16).astype(jnp.float32)
        sc = jax.nn.sigmoid(zz).astype(jnp.bfloat16).astype(jnp.float32)
        scale_ref[...] = jnp.broadcast_to(sc, scale_ref.shape)

        osem = sems.at[0]

        def obody(t, carry):
            for cb in range(C // KW):
                rows = pl.ds(cb * KW, KW)
                sc = scale_ref[rows, :]
                for s in range(S):
                    v = buf[s, t, rows, :].astype(jnp.float32) * sc
                    buf[s, t, rows, :] = v.astype(jnp.bfloat16)
                idx = (slice(None), pl.ds(t, 1), rows)
                pltpu.make_async_copy(buf.at[idx], o_hbm.at[idx], osem).start()
            return carry

        jax.lax.fori_loop(0, Hs, obody, 0)
        pltpu.make_async_copy(buf, o_hbm, osem).wait()

    xt = jnp.transpose(x, (0, 1, 3, 2)).reshape(shp)
    o = pl.pallas_call(
        kernel,
        out_shape=jax.ShapeDtypeStruct(shp, x.dtype),
        in_specs=[pl.BlockSpec(memory_space=pl.ANY)] * 3,
        out_specs=pl.BlockSpec(memory_space=pl.ANY),
        scratch_shapes=[
            pltpu.VMEM(shp, x.dtype),
            pltpu.VMEM((R, C), w1.dtype),
            pltpu.VMEM((R, C), w2.dtype),
            pltpu.VMEM((C, W), jnp.float32),
            pltpu.VMEM((C, W), jnp.float32),
            pltpu.VMEM((C, W), jnp.float32),
            pltpu.SemaphoreType.DMA((D + 1,)),
        ],
        compiler_params=pltpu.CompilerParams(vmem_limit_bytes=64 * 1024 * 1024),
    )(xt, w1.T, w2)
    return jnp.transpose(o.reshape(B, H, C, W), (0, 1, 3, 2))
```

```python
import jax
import jax.numpy as jnp
import jax.experimental.pallas as pl
import jax.experimental.pallas.tpu as pltpu

F32 = jnp.float32
BF16 = jnp.bfloat16

S = 7
P = 2048
K = 32
D = 4
TAIL = (2, 2, 1, 1)


def _rnd(v):
    return v.astype(BF16).astype(F32)


@jax.jit
def pallas_standalone__channel_attn_cbam__vision_kernel(
    x: jax.Array,
    w1: jax.Array,
    w2: jax.Array,
):
    Bn, H, W, C = x.shape
    R = w1.shape[1]
    rows_total = H * C
    G = rows_total // (S * P)
    NB = P // K
    NC = C // K
    T = G * NB
    NG = T // NC
    sh = NB % NC
    assert Bn == 1 and G * S * P == rows_total and P % K == 0 and C % K == 0
    assert T % NC == 0 and ((S - 1) * NB) % NC == 0 and NB & (NB - 1) == 0
    assert sum(TAIL) == NC and NG - 1 - D >= 1 and R <= 64 and 128 < W <= 256
    log_nb = NB.bit_length() - 1
    shp = (G, S, NB, K, W)
    inv_n = 1.0 / (H * W)

    def gb(tau):
        if isinstance(tau, int):
            return tau // NB, tau % NB
        return (jax.lax.shift_right_logical(tau, log_nb),
                jax.lax.bitwise_and(tau, NB - 1))

    def jof(cg, s):
        return (cg - sh * s) % NC

    def kernel(x_hbm, w1t_hbm, w2_hbm, o_hbm, buf, w1t_v, w2_v, w1d_ref, w2d_ref,
               sum_ref, max_ref, scale_ref, sems):
        def rd(g, s, b, slot):
            idx = (pl.ds(g, 1), pl.ds(s, 1), pl.ds(b, 1))
            return pltpu.make_async_copy(x_hbm.at[idx], buf.at[idx], sems.at[slot])

        def group_blocks(i):
            out = []
            for j in range(NC):
                g, b = gb(i * NC + j)
                out += [(g, s, b) for s in range(S)]
            return out

        def tail_blocks(cgs):
            out = []
            for cg in cgs:
                for s in range(S):
                    g, b = gb((NG - 1) * NC + jof(cg, s))
                    out.append((g, s, b))
            return out

        def start(blocks, slot):
            for (g, s, b) in blocks:
                rd(g, s, b, slot).start(priority=int(s > 0))

        def wait(blocks, slot):
            for (g, s, b) in blocks:
                rd(g, s, b, slot).wait()

        def block_reduce(i, cg):
            sa = ma = None
            for s in range(S):
                g, b = gb(i * NC + jof(cg, s))
                v = buf[g, s, b].astype(F32)
                sa = v if sa is None else sa + v
                ma = v if ma is None else jnp.maximum(ma, v)
            return sa, ma

        def accumulate(i, first=False):
            for cg in range(NC):
                rows = pl.ds(cg * K, K)
                sa, ma = block_reduce(i, cg)
                if first:
                    sum_ref[rows, :] = sa
                    max_ref[rows, :] = ma
                else:
                    sum_ref[rows, :] = sum_ref[rows, :] + sa
                    max_ref[rows, :] = jnp.maximum(max_ref[rows, :], ma)

        start(group_blocks(0), 0)
        cw1 = pltpu.make_async_copy(w1t_hbm, w1t_v, sems.at[0])
        cw2 = pltpu.make_async_copy(w2_hbm, w2_v, sems.at[0])
        cw1.start()
        cw2.start()
        for i in range(1, D):
            start(group_blocks(i), i)

        wait(group_blocks(0), 0)
        cw1.wait()
        cw2.wait()
        start(group_blocks(D), 0)
        accumulate(0, first=True)
        jj = jax.lax.broadcasted_iota(jnp.int32, (R, 128), 0)
        ll = jax.lax.broadcasted_iota(jnp.int32, (R, 128), 1)
        sel = jnp.where((ll == jj) | (ll == jj + 64), 1.0, 0.0).astype(BF16)
        dn = (((0,), (0,)), ((), ()))
        w1d_ref[...] = jax.lax.dot_general(w1t_v[...], sel, dn, preferred_element_type=F32)
        w2d_ref[...] = jax.lax.dot_general(w2_v[...], sel, dn, preferred_element_type=F32)

        def body(i, carry):
            slot = jax.lax.rem(i, D)
            wait(group_blocks(i), slot)
            start(group_blocks(i + D), slot)
            accumulate(i)
            return carry

        nfull = NG - 1
        jax.lax.fori_loop(1, nfull - D, body, 0)

        offs = [sum(TAIL[:i]) for i in range(len(TAIL) + 1)]
        pieces = [tuple(range(offs[i], offs[i + 1])) for i in range(len(TAIL))]
        rest = [(i, None) for i in range(nfull - D, nfull)] + [(NG - 1, pc) for pc in pieces]
        hpart = jnp.zeros((8, 128), F32)
        for k, (i, pc) in enumerate(rest):
            slot = (nfull - D + k) % D
            wait(group_blocks(i) if pc is None else tail_blocks(pc), slot)
            if k + D < len(rest):
                i2, pc2 = rest[k + D]
                start(group_blocks(i2) if pc2 is None else tail_blocks(pc2), slot)
            if pc is None:
                accumulate(i)
                continue
            for cg in pc:
                rows = pl.ds(cg * K, K)
                sa, ma = block_reduce(i, cg)
                tot = sum_ref[rows, :] + sa
                mx = jnp.maximum(max_ref[rows, :], ma)
                gap = jnp.broadcast_to(jnp.sum(tot, axis=1, keepdims=True), (K, 128))
                gap = _rnd(gap * inv_n)
                gmp = jnp.broadcast_to(jnp.max(mx, axis=1, keepdims=True), (K, 128))
                lane = jax.lax.broadcasted_iota(jnp.int32, (K, 128), 1)
                pr = jnp.where(lane < 64, gap, gmp) * w1d_ref[rows, :]
                for r in range(K // 8):
                    hpart = hpart + pr[r * 8:(r + 1) * 8, :]

        osem = sems.at[0]

        def scale_blk(g, s, b, sc):
            buf[g, s, b] = (buf[g, s, b].astype(F32) * sc).astype(BF16)

        def wr(g, s0, s1, b):
            idx = (pl.ds(g, 1), pl.ds(s0, s1 - s0), pl.ds(b, 1))
            pltpu.make_async_copy(buf.at[idx], o_hbm.at[idx], osem).start()

        h = jnp.sum(hpart, axis=0, keepdims=True)
        h = jnp.maximum(_rnd(h), 0.0)
        for cg in range(NC):
            rows = pl.ds(cg * K, K)
            z = jnp.sum(w2d_ref[rows, :] * h, axis=1, keepdims=True)
            z = _rnd(jnp.broadcast_to(z, (K, 128)))
            sc = _rnd(jax.nn.sigmoid(z))
            sc = jnp.concatenate([sc, sc[:, :W - 128]], axis=1)
            scale_ref[rows, :] = sc
            for s in range(S):
                g, b = gb(jof(cg, s))
                scale_blk(g, s, b, sc)
                wr(g, s, s + 1, b)

        def obody(i, carry):
            for j in range(NC):
                g, b = gb(i * NC + j)
                for s in range(S):
                    cg = (j + sh * s) % NC
                    scale_blk(g, s, b, scale_ref[pl.ds(cg * K, K), :])
                wr(g, 0, S, b)
            return carry

        jax.lax.fori_loop(1, NG, obody, 0)
        pltpu.make_async_copy(buf, o_hbm, osem).wait()

    xt = jnp.transpose(x, (0, 1, 3, 2)).reshape(shp)
    o = pl.pallas_call(
        kernel,
        out_shape=jax.ShapeDtypeStruct(shp, x.dtype),
        in_specs=[pl.BlockSpec(memory_space=pl.ANY)] * 3,
        out_specs=pl.BlockSpec(memory_space=pl.ANY),
        scratch_shapes=[
            pltpu.VMEM(shp, x.dtype),
            pltpu.VMEM((R, C), w1.dtype),
            pltpu.VMEM((R, C), w2.dtype),
            pltpu.VMEM((C, 128), F32),
            pltpu.VMEM((C, 128), F32),
            pltpu.VMEM((C, W), F32),
            pltpu.VMEM((C, W), F32),
            pltpu.VMEM((C, W), F32),
            pltpu.SemaphoreType.DMA((D,)),
        ],
        compiler_params=pltpu.CompilerParams(
            vmem_limit_bytes=64 * 1024 * 1024, disable_bounds_checks=True),
    )(xt, w1.T, w2)
    return jnp.transpose(o.reshape(Bn, H, C, W), (0, 1, 3, 2))
```

```python
import jax
import jax.numpy as jnp
import jax.experimental.pallas as pl
import jax.experimental.pallas.tpu as pltpu

F32 = jnp.float32
BF16 = jnp.bfloat16

S = 7
P = 2048
K = 32
D = 4
TAIL = (2, 2, 1, 1)

_COMPILER_PARAMS = dict(vmem_limit_bytes=64 * 1024 * 1024)
for _opt in ("disable_bounds_checks", "disable_semaphore_checks"):
    if hasattr(pltpu.CompilerParams, _opt):
        _COMPILER_PARAMS[_opt] = True


def _rnd(v):
    return v.astype(BF16).astype(F32)


@jax.jit
def pallas_standalone__channel_attn_cbam__vision_kernel(
    x: jax.Array,
    w1: jax.Array,
    w2: jax.Array,
):
    Bn, H, W, C = x.shape
    R = w1.shape[1]
    rows_total = H * C
    G = rows_total // (S * P)
    NB = P // K
    NC = C // K
    T = G * NB
    NG = T // NC
    sh = NB % NC
    assert Bn == 1 and G * S * P == rows_total and P % K == 0 and C % K == 0
    assert T % NC == 0 and ((S - 1) * NB) % NC == 0 and NB & (NB - 1) == 0
    assert sum(TAIL) == NC and NG - 1 - D >= 1 and R <= 64 and 128 < W <= 256
    log_nb = NB.bit_length() - 1
    shp = (G, S, NB, K, W)
    inv_n = 1.0 / (H * W)

    def gb(tau):
        if isinstance(tau, int):
            return tau // NB, tau % NB
        return (jax.lax.shift_right_logical(tau, log_nb),
                jax.lax.bitwise_and(tau, NB - 1))

    def jof(cg, s):
        return (cg - sh * s) % NC

    def kernel(x_hbm, w1t_hbm, w2_hbm, o_hbm, buf, w1t_v, w2_v, w1d_ref, w2d_ref,
               sum_ref, max_ref, scale_ref, sems):
        def rd(g, s, b, slot):
            idx = (pl.ds(g, 1), pl.ds(s, 1), pl.ds(b, 1))
            return pltpu.make_async_copy(x_hbm.at[idx], buf.at[idx], sems.at[slot])

        def group_blocks(i):
            out = []
            for j in range(NC):
                g, b = gb(i * NC + j)
                out += [(g, s, b) for s in range(S)]
            return out

        def tail_blocks(cgs):
            out = []
            for cg in cgs:
                for s in range(S):
                    g, b = gb((NG - 1) * NC + jof(cg, s))
                    out.append((g, s, b))
            return out

        def start(blocks, slot):
            for (g, s, b) in blocks:
                rd(g, s, b, slot).start(priority=int(s > 0))

        def wait(blocks, slot):
            for (g, s, b) in blocks:
                rd(g, s, b, slot).wait()

        def block_reduce(i, cg):
            sa = ma = None
            for s in range(S):
                g, b = gb(i * NC + jof(cg, s))
                v = buf[g, s, b].astype(F32)
                sa = v if sa is None else sa + v
                ma = v if ma is None else jnp.maximum(ma, v)
            return sa, ma

        def accumulate(i, first=False):
            for cg in range(NC):
                rows = pl.ds(cg * K, K)
                sa, ma = block_reduce(i, cg)
                if first:
                    sum_ref[rows, :] = sa
                    max_ref[rows, :] = ma
                else:
                    sum_ref[rows, :] = sum_ref[rows, :] + sa
                    max_ref[rows, :] = jnp.maximum(max_ref[rows, :], ma)

        start(group_blocks(0), 0)
        cw1 = pltpu.make_async_copy(w1t_hbm, w1t_v, sems.at[0])
        cw2 = pltpu.make_async_copy(w2_hbm, w2_v, sems.at[0])
        cw1.start()
        cw2.start()
        for i in range(1, D):
            start(group_blocks(i), i)

        wait(group_blocks(0), 0)
        cw1.wait()
        cw2.wait()
        start(group_blocks(D), 0)
        accumulate(0, first=True)
        jj = jax.lax.broadcasted_iota(jnp.int32, (R, 128), 0)
        ll = jax.lax.broadcasted_iota(jnp.int32, (R, 128), 1)
        sel = jnp.where((ll == jj) | (ll == jj + 64), 1.0, 0.0).astype(BF16)
        dn = (((0,), (0,)), ((), ()))
        w1d_ref[...] = jax.lax.dot_general(w1t_v[...], sel, dn, preferred_element_type=F32)
        w2d_ref[...] = jax.lax.dot_general(w2_v[...], sel, dn, preferred_element_type=F32)

        def body(i, carry):
            slot = jax.lax.rem(i, D)
            wait(group_blocks(i), slot)
            start(group_blocks(i + D), slot)
            accumulate(i)
            return carry

        nfull = NG - 1
        jax.lax.fori_loop(1, nfull - D, body, 0)

        offs = [sum(TAIL[:i]) for i in range(len(TAIL) + 1)]
        pieces = [tuple(range(offs[i], offs[i + 1])) for i in range(len(TAIL))]
        rest = [(i, None) for i in range(nfull - D, nfull)] + [(NG - 1, pc) for pc in pieces]
        hpart = jnp.zeros((8, 128), F32)
        for k, (i, pc) in enumerate(rest):
            slot = (nfull - D + k) % D
            wait(group_blocks(i) if pc is None else tail_blocks(pc), slot)
            if k + D < len(rest):
                i2, pc2 = rest[k + D]
                start(group_blocks(i2) if pc2 is None else tail_blocks(pc2), slot)
            if pc is None:
                accumulate(i)
                continue
            for cg in pc:
                rows = pl.ds(cg * K, K)
                sa, ma = block_reduce(i, cg)
                tot = sum_ref[rows, :] + sa
                mx = jnp.maximum(max_ref[rows, :], ma)
                gap = jnp.broadcast_to(jnp.sum(tot, axis=1, keepdims=True), (K, 128))
                gap = _rnd(gap * inv_n)
                gmp = jnp.broadcast_to(jnp.max(mx, axis=1, keepdims=True), (K, 128))
                lane = jax.lax.broadcasted_iota(jnp.int32, (K, 128), 1)
                pr = jnp.where(lane < 64, gap, gmp) * w1d_ref[rows, :]
                for r in range(K // 8):
                    hpart = hpart + pr[r * 8:(r + 1) * 8, :]

        osem = sems.at[0]

        def scale_blk(g, s, b, sc):
            buf[g, s, b] = (buf[g, s, b].astype(F32) * sc).astype(BF16)

        def wr(g, s0, s1, b):
            idx = (pl.ds(g, 1), pl.ds(s0, s1 - s0), pl.ds(b, 1))
            pltpu.make_async_copy(buf.at[idx], o_hbm.at[idx], osem).start()

        h = jnp.sum(hpart, axis=0, keepdims=True)
        h = jnp.maximum(_rnd(h), 0.0)
        for cg in range(NC):
            rows = pl.ds(cg * K, K)
            z = jnp.sum(w2d_ref[rows, :] * h, axis=1, keepdims=True)
            z = _rnd(jnp.broadcast_to(z, (K, 128)))
            sc = _rnd(jax.nn.sigmoid(z))
            sc = jnp.concatenate([sc, sc[:, :W - 128]], axis=1)
            scale_ref[rows, :] = sc
            for s in range(S):
                g, b = gb(jof(cg, s))
                scale_blk(g, s, b, sc)
                wr(g, s, s + 1, b)

        def obody(i, carry):
            for j in range(NC):
                g, b = gb(i * NC + j)
                for s in range(S):
                    cg = (j + sh * s) % NC
                    scale_blk(g, s, b, scale_ref[pl.ds(cg * K, K), :])
                wr(g, 0, S, b)
            return carry

        jax.lax.fori_loop(1, NG, obody, 0)
        pltpu.make_async_copy(buf, o_hbm, osem).wait()

    xt = jnp.transpose(x, (0, 1, 3, 2)).reshape(shp)
    o = pl.pallas_call(
        kernel,
        out_shape=jax.ShapeDtypeStruct(shp, x.dtype),
        in_specs=[pl.BlockSpec(memory_space=pl.ANY)] * 3,
        out_specs=pl.BlockSpec(memory_space=pl.ANY),
        scratch_shapes=[
            pltpu.VMEM(shp, x.dtype),
            pltpu.VMEM((R, C), w1.dtype),
            pltpu.VMEM((R, C), w2.dtype),
            pltpu.VMEM((C, 128), F32),
            pltpu.VMEM((C, 128), F32),
            pltpu.VMEM((C, W), F32),
            pltpu.VMEM((C, W), F32),
            pltpu.VMEM((C, W), F32),
            pltpu.SemaphoreType.DMA((D,)),
        ],
        compiler_params=pltpu.CompilerParams(**_COMPILER_PARAMS),
    )(xt, w1.T, w2)
    return jnp.transpose(o.reshape(Bn, H, C, W), (0, 1, 3, 2))
```

```python
import jax
import jax.numpy as jnp
import jax.experimental.pallas as pl
import jax.experimental.pallas.tpu as pltpu

F32 = jnp.float32
BF16 = jnp.bfloat16

S = 7
P = 2048
K = 32
KD = 8
D = 4
TAIL = (2, 2, 1, 1)

_COMPILER_PARAMS = dict(vmem_limit_bytes=64 * 1024 * 1024)
for _opt in ("disable_bounds_checks", "disable_semaphore_checks"):
    if hasattr(pltpu.CompilerParams, _opt):
        _COMPILER_PARAMS[_opt] = True


def _rnd(v):
    return v.astype(BF16).astype(F32)


@jax.jit
def pallas_standalone__channel_attn_cbam__vision_kernel(
    x: jax.Array,
    w1: jax.Array,
    w2: jax.Array,
):
    Bn, H, W, C = x.shape
    R = w1.shape[1]
    rows_total = H * C
    G = rows_total // (S * P)
    NB = P // K
    NC = C // K
    T = G * NB
    NG = T // NC
    sh = NB % NC
    assert Bn == 1 and G * S * P == rows_total and P % K == 0 and C % K == 0 and K % KD == 0
    assert T % NC == 0 and ((S - 1) * NB) % NC == 0 and NB & (NB - 1) == 0
    assert sum(TAIL) == NC and NG - 1 - D >= 1 and R <= 64 and 128 < W <= 256
    log_nb = NB.bit_length() - 1
    shp = (G, S, NB, K, W)
    inv_n = 1.0 / (H * W)

    def gb(tau):
        if isinstance(tau, int):
            return tau // NB, tau % NB
        return (jax.lax.shift_right_logical(tau, log_nb),
                jax.lax.bitwise_and(tau, NB - 1))

    def jof(cg, s):
        return (cg - sh * s) % NC

    def kernel(x_hbm, w1t_hbm, w2_hbm, o_hbm, buf, w1t_v, w2_v, w1d_ref, w2d_ref,
               sum_ref, max_ref, scale_ref, sems):
        def rd(g, s, b, r0, slot):
            idx = (pl.ds(g, 1), pl.ds(s, 1), pl.ds(b, 1), pl.ds(r0, KD))
            return pltpu.make_async_copy(x_hbm.at[idx], buf.at[idx], sems.at[slot])

        def group_copies(i):
            out = []
            for j in range(NC):
                g, b = gb(i * NC + j)
                out += [(g, s, b, r0) for r0 in range(0, K, KD) for s in range(S)]
            return out

        def tail_copies(cgs):
            out = []
            for cg in cgs:
                for r0 in range(0, K, KD):
                    for s in range(S):
                        g, b = gb((NG - 1) * NC + jof(cg, s))
                        out.append((g, s, b, r0))
            return out

        def start(copies, slot):
            for (g, s, b, r0) in copies:
                rd(g, s, b, r0, slot).start(priority=int(s > 0))

        def wait(copies, slot):
            for (g, s, b, r0) in copies:
                rd(g, s, b, r0, slot).wait()

        def block_reduce(i, cg):
            sa = ma = None
            for s in range(S):
                g, b = gb(i * NC + jof(cg, s))
                v = buf[g, s, b].astype(F32)
                sa = v if sa is None else sa + v
                ma = v if ma is None else jnp.maximum(ma, v)
            return sa, ma

        def accumulate(i, first=False):
            for cg in range(NC):
                rows = pl.ds(cg * K, K)
                sa, ma = block_reduce(i, cg)
                if first:
                    sum_ref[rows, :] = sa
                    max_ref[rows, :] = ma
                else:
                    sum_ref[rows, :] = sum_ref[rows, :] + sa
                    max_ref[rows, :] = jnp.maximum(max_ref[rows, :], ma)

        start(group_copies(0), 0)
        cw1 = pltpu.make_async_copy(w1t_hbm, w1t_v, sems.at[0])
        cw2 = pltpu.make_async_copy(w2_hbm, w2_v, sems.at[0])
        cw1.start()
        cw2.start()
        for i in range(1, D):
            start(group_copies(i), i)

        wait(group_copies(0), 0)
        cw1.wait()
        cw2.wait()
        start(group_copies(D), 0)
        accumulate(0, first=True)
        jj = jax.lax.broadcasted_iota(jnp.int32, (R, 128), 0)
        ll = jax.lax.broadcasted_iota(jnp.int32, (R, 128), 1)
        sel = jnp.where((ll == jj) | (ll == jj + 64), 1.0, 0.0).astype(BF16)
        dn = (((0,), (0,)), ((), ()))
        w1d_ref[...] = jax.lax.dot_general(w1t_v[...], sel, dn, preferred_element_type=F32)
        w2d_ref[...] = jax.lax.dot_general(w2_v[...], sel, dn, preferred_element_type=F32)

        def body(i, carry):
            slot = jax.lax.rem(i, D)
            wait(group_copies(i), slot)
            accumulate(i)
            start(group_copies(i + D), slot)
            return carry

        nfull = NG - 1
        jax.lax.fori_loop(1, nfull - D, body, 0)

        offs = [sum(TAIL[:i]) for i in range(len(TAIL) + 1)]
        pieces = [tuple(range(offs[i], offs[i + 1])) for i in range(len(TAIL))]
        rest = [(i, None) for i in range(nfull - D, nfull)] + [(NG - 1, pc) for pc in pieces]
        hpart = jnp.zeros((8, 128), F32)
        for k, (i, pc) in enumerate(rest):
            slot = (nfull - D + k) % D
            wait(group_copies(i) if pc is None else tail_copies(pc), slot)
            if pc is None:
                accumulate(i)
            if k + D < len(rest):
                i2, pc2 = rest[k + D]
                start(group_copies(i2) if pc2 is None else tail_copies(pc2), slot)
            if pc is None:
                continue
            for cg in pc:
                rows = pl.ds(cg * K, K)
                sa, ma = block_reduce(i, cg)
                tot = sum_ref[rows, :] + sa
                mx = jnp.maximum(max_ref[rows, :], ma)
                gap = jnp.broadcast_to(jnp.sum(tot, axis=1, keepdims=True), (K, 128))
                gap = _rnd(gap * inv_n)
                gmp = jnp.broadcast_to(jnp.max(mx, axis=1, keepdims=True), (K, 128))
                lane = jax.lax.broadcasted_iota(jnp.int32, (K, 128), 1)
                pr = jnp.where(lane < 64, gap, gmp) * w1d_ref[rows, :]
                for r in range(K // 8):
                    hpart = hpart + pr[r * 8:(r + 1) * 8, :]

        osem = sems.at[0]

        def scale_blk(g, s, b, sc):
            buf[g, s, b] = (buf[g, s, b].astype(F32) * sc).astype(BF16)

        def wr(g, s0, s1, b):
            idx = (pl.ds(g, 1), pl.ds(s0, s1 - s0), pl.ds(b, 1))
            pltpu.make_async_copy(buf.at[idx], o_hbm.at[idx], osem).start()

        h = jnp.sum(hpart, axis=0, keepdims=True)
        h = jnp.maximum(_rnd(h), 0.0)
        for cg in range(NC):
            rows = pl.ds(cg * K, K)
            z = jnp.sum(w2d_ref[rows, :] * h, axis=1, keepdims=True)
            z = _rnd(jnp.broadcast_to(z, (K, 128)))
            sc = _rnd(jax.nn.sigmoid(z))
            sc = jnp.concatenate([sc, sc[:, :W - 128]], axis=1)
            scale_ref[rows, :] = sc
            for s in range(S):
                g, b = gb(jof(cg, s))
                scale_blk(g, s, b, sc)
                wr(g, s, s + 1, b)

        def obody(i, carry):
            for j in range(NC):
                g, b = gb(i * NC + j)
                for s in range(S):
                    cg = (j + sh * s) % NC
                    scale_blk(g, s, b, scale_ref[pl.ds(cg * K, K), :])
                wr(g, 0, S, b)
            return carry

        jax.lax.fori_loop(1, NG, obody, 0)
        pltpu.make_async_copy(buf, o_hbm, osem).wait()

    xt = jnp.transpose(x, (0, 1, 3, 2)).reshape(shp)
    o = pl.pallas_call(
        kernel,
        out_shape=jax.ShapeDtypeStruct(shp, x.dtype),
        in_specs=[pl.BlockSpec(memory_space=pl.ANY)] * 3,
        out_specs=pl.BlockSpec(memory_space=pl.ANY),
        scratch_shapes=[
            pltpu.VMEM(shp, x.dtype),
            pltpu.VMEM((R, C), w1.dtype),
            pltpu.VMEM((R, C), w2.dtype),
            pltpu.VMEM((C, 128), F32),
            pltpu.VMEM((C, 128), F32),
            pltpu.VMEM((C, W), F32),
            pltpu.VMEM((C, W), F32),
            pltpu.VMEM((C, W), F32),
            pltpu.SemaphoreType.DMA((D,)),
        ],
        compiler_params=pltpu.CompilerParams(**_COMPILER_PARAMS),
    )(xt, w1.T, w2)
    return jnp.transpose(o.reshape(Bn, H, C, W), (0, 1, 3, 2))
```

```python
import jax
import jax.numpy as jnp
import jax.experimental.pallas as pl
import jax.experimental.pallas.tpu as pltpu

F32 = jnp.float32
BF16 = jnp.bfloat16

S = 7
P = 2048
K = 32
KD = 16
PARTS = ((0, 1, 0), (1, 4, 1), (4, 7, 1))
D = 4
TAIL = (2, 2, 1, 1)

_COMPILER_PARAMS = dict(vmem_limit_bytes=64 * 1024 * 1024)
for _opt in ("disable_bounds_checks", "disable_semaphore_checks"):
    if hasattr(pltpu.CompilerParams, _opt):
        _COMPILER_PARAMS[_opt] = True


def _rnd(v):
    return v.astype(BF16).astype(F32)


@jax.jit
def pallas_standalone__channel_attn_cbam__vision_kernel(
    x: jax.Array,
    w1: jax.Array,
    w2: jax.Array,
):
    Bn, H, W, C = x.shape
    R = w1.shape[1]
    rows_total = H * C
    G = rows_total // (S * P)
    NB = P // K
    NC = C // K
    T = G * NB
    NG = T // NC
    sh = NB % NC
    assert Bn == 1 and G * S * P == rows_total and P % K == 0 and C % K == 0 and K % KD == 0
    assert T % NC == 0 and ((S - 1) * NB) % NC == 0 and NB & (NB - 1) == 0
    assert sum(TAIL) == NC and NG - 1 - D >= 1 and R <= 64 and 128 < W <= 256
    assert [p[0] for p in PARTS] + [S] == [0] + [p[1] for p in PARTS]
    log_nb = NB.bit_length() - 1
    shp = (G, S, NB, K, W)
    inv_n = 1.0 / (H * W)

    def gb(tau):
        if isinstance(tau, int):
            return tau // NB, tau % NB
        return (jax.lax.shift_right_logical(tau, log_nb),
                jax.lax.bitwise_and(tau, NB - 1))

    def jof(cg, s):
        return (cg - sh * s) % NC

    def kernel(x_hbm, w1t_hbm, w2_hbm, o_hbm, buf, w1t_v, w2_v, w1d_ref, w2d_ref,
               sum_ref, max_ref, scale_ref, sems):
        def rd(g, s0, s1, b, r0, nr, slot):
            idx = (pl.ds(g, 1), pl.ds(s0, s1 - s0), pl.ds(b, 1), pl.ds(r0, nr))
            return pltpu.make_async_copy(x_hbm.at[idx], buf.at[idx], sems.at[slot])

        def group_copies(i):
            out = []
            for j in range(NC):
                g, b = gb(i * NC + j)
                out += [((g, s0, s1, b, r0, KD), prio)
                        for r0 in range(0, K, KD) for (s0, s1, prio) in PARTS]
            return out

        def tail_copies(cgs):
            out = []
            for cg in cgs:
                for s in range(S):
                    g, b = gb((NG - 1) * NC + jof(cg, s))
                    out.append(((g, s, s + 1, b, 0, K), int(s > 0)))
            return out

        def start(copies, slot):
            for (args, prio) in copies:
                rd(*args, slot).start(priority=prio)

        def wait(copies, slot):
            for (args, _) in copies:
                rd(*args, slot).wait()

        def block_reduce(i, cg):
            sa = ma = None
            for s in range(S):
                g, b = gb(i * NC + jof(cg, s))
                v = buf[g, s, b].astype(F32)
                sa = v if sa is None else sa + v
                ma = v if ma is None else jnp.maximum(ma, v)
            return sa, ma

        def accumulate(i, first=False):
            for cg in range(NC):
                rows = pl.ds(cg * K, K)
                sa, ma = block_reduce(i, cg)
                if first:
                    sum_ref[rows, :] = sa
                    max_ref[rows, :] = ma
                else:
                    sum_ref[rows, :] = sum_ref[rows, :] + sa
                    max_ref[rows, :] = jnp.maximum(max_ref[rows, :], ma)

        start(group_copies(0), 0)
        cw1 = pltpu.make_async_copy(w1t_hbm, w1t_v, sems.at[0])
        cw2 = pltpu.make_async_copy(w2_hbm, w2_v, sems.at[0])
        cw1.start()
        cw2.start()
        for i in range(1, D):
            start(group_copies(i), i)

        wait(group_copies(0), 0)
        cw1.wait()
        cw2.wait()
        start(group_copies(D), 0)
        accumulate(0, first=True)
        jj = jax.lax.broadcasted_iota(jnp.int32, (R, 128), 0)
        ll = jax.lax.broadcasted_iota(jnp.int32, (R, 128), 1)
        sel = jnp.where((ll == jj) | (ll == jj + 64), 1.0, 0.0).astype(BF16)
        dn = (((0,), (0,)), ((), ()))
        w1d_ref[...] = jax.lax.dot_general(w1t_v[...], sel, dn, preferred_element_type=F32)
        w2d_ref[...] = jax.lax.dot_general(w2_v[...], sel, dn, preferred_element_type=F32)

        def body(i, carry):
            slot = jax.lax.rem(i, D)
            wait(group_copies(i), slot)
            start(group_copies(i + D), slot)
            accumulate(i)
            return carry

        nfull = NG - 1
        jax.lax.fori_loop(1, nfull - D, body, 0)

        offs = [sum(TAIL[:i]) for i in range(len(TAIL) + 1)]
        pieces = [tuple(range(offs[i], offs[i + 1])) for i in range(len(TAIL))]
        rest = [(i, None) for i in range(nfull - D, nfull)] + [(NG - 1, pc) for pc in pieces]
        hpart = jnp.zeros((8, 128), F32)
        for k, (i, pc) in enumerate(rest):
            slot = (nfull - D + k) % D
            wait(group_copies(i) if pc is None else tail_copies(pc), slot)
            if k + D < len(rest):
                i2, pc2 = rest[k + D]
                start(group_copies(i2) if pc2 is None else tail_copies(pc2), slot)
            if pc is None:
                accumulate(i)
                continue
            for cg in pc:
                rows = pl.ds(cg * K, K)
                sa, ma = block_reduce(i, cg)
                tot = sum_ref[rows, :] + sa
                mx = jnp.maximum(max_ref[rows, :], ma)
                gap = jnp.broadcast_to(jnp.sum(tot, axis=1, keepdims=True), (K, 128))
                gap = _rnd(gap * inv_n)
                gmp = jnp.broadcast_to(jnp.max(mx, axis=1, keepdims=True), (K, 128))
                lane = jax.lax.broadcasted_iota(jnp.int32, (K, 128), 1)
                pr = jnp.where(lane < 64, gap, gmp) * w1d_ref[rows, :]
                for r in range(K // 8):
                    hpart = hpart + pr[r * 8:(r + 1) * 8, :]

        osem = sems.at[0]

        def scale_blk(g, s, b, sc):
            buf[g, s, b] = (buf[g, s, b].astype(F32) * sc).astype(BF16)

        def wr(g, s0, s1, b):
            idx = (pl.ds(g, 1), pl.ds(s0, s1 - s0), pl.ds(b, 1))
            pltpu.make_async_copy(buf.at[idx], o_hbm.at[idx], osem).start()

        h = jnp.sum(hpart, axis=0, keepdims=True)
        h = jnp.maximum(_rnd(h), 0.0)
        for cg in range(NC):
            rows = pl.ds(cg * K, K)
            z = jnp.sum(w2d_ref[rows, :] * h, axis=1, keepdims=True)
            z = _rnd(jnp.broadcast_to(z, (K, 128)))
            sc = _rnd(jax.nn.sigmoid(z))
            sc = jnp.concatenate([sc, sc[:, :W - 128]], axis=1)
            scale_ref[rows, :] = sc
            for s in range(S):
                g, b = gb(jof(cg, s))
                scale_blk(g, s, b, sc)
                wr(g, s, s + 1, b)

        def obody(i, carry):
            for j in range(NC):
                g, b = gb(i * NC + j)
                for s in range(S):
                    cg = (j + sh * s) % NC
                    scale_blk(g, s, b, scale_ref[pl.ds(cg * K, K), :])
                wr(g, 0, S, b)
            return carry

        jax.lax.fori_loop(1, NG, obody, 0)
        pltpu.make_async_copy(buf, o_hbm, osem).wait()

    xt = jnp.transpose(x, (0, 1, 3, 2)).reshape(shp)
    o = pl.pallas_call(
        kernel,
        out_shape=jax.ShapeDtypeStruct(shp, x.dtype),
        in_specs=[pl.BlockSpec(memory_space=pl.ANY)] * 3,
        out_specs=pl.BlockSpec(memory_space=pl.ANY),
        scratch_shapes=[
            pltpu.VMEM(shp, x.dtype),
            pltpu.VMEM((R, C), w1.dtype),
            pltpu.VMEM((R, C), w2.dtype),
            pltpu.VMEM((C, 128), F32),
            pltpu.VMEM((C, 128), F32),
            pltpu.VMEM((C, W), F32),
            pltpu.VMEM((C, W), F32),
            pltpu.VMEM((C, W), F32),
            pltpu.SemaphoreType.DMA((D,)),
        ],
        compiler_params=pltpu.CompilerParams(**_COMPILER_PARAMS),
    )(xt, w1.T, w2)
    return jnp.transpose(o.reshape(Bn, H, C, W), (0, 1, 3, 2))
```

```python
import jax
import jax.numpy as jnp
import jax.experimental.pallas as pl
import jax.experimental.pallas.tpu as pltpu

F32 = jnp.float32
BF16 = jnp.bfloat16

S = 7
P = 2048
K = 32
KD = 16
PARTS = ((0, 1, 0), (1, 4, 1), (4, 7, 1))
D = 4
TAIL = (2, 2, 1, 1)

_COMPILER_PARAMS = dict(vmem_limit_bytes=64 * 1024 * 1024)
for _opt in ("disable_bounds_checks", "disable_semaphore_checks"):
    if hasattr(pltpu.CompilerParams, _opt):
        _COMPILER_PARAMS[_opt] = True


def _rnd(v):
    return v.astype(BF16).astype(F32)


@jax.jit
def pallas_standalone__channel_attn_cbam__vision_kernel(
    x: jax.Array,
    w1: jax.Array,
    w2: jax.Array,
):
    Bn, H, W, C = x.shape
    R = w1.shape[1]
    rows_total = H * C
    G = rows_total // (S * P)
    NB = P // K
    NC = C // K
    T = G * NB
    NG = T // NC
    sh = NB % NC
    assert Bn == 1 and G * S * P == rows_total and P % K == 0 and C % K == 0 and K % KD == 0
    assert T % NC == 0 and ((S - 1) * NB) % NC == 0 and NB & (NB - 1) == 0
    assert sum(TAIL) == NC and NG - 1 - D >= 1 and R <= 64 and 128 < W <= 256
    assert [p[0] for p in PARTS] + [S] == [0] + [p[1] for p in PARTS]
    log_nb = NB.bit_length() - 1
    shp = (G, S, NB, K, W)
    inv_n = 1.0 / (H * W)

    def gb(tau):
        if isinstance(tau, int):
            return tau // NB, tau % NB
        return (jax.lax.shift_right_logical(tau, log_nb),
                jax.lax.bitwise_and(tau, NB - 1))

    def jof(cg, s):
        return (cg - sh * s) % NC

    def kernel(x_hbm, w1t_hbm, w2_hbm, o_hbm, buf, w1t_v, w2_v, w1d_ref, w2d_ref,
               sum_ref, max_ref, scale_ref, sems):
        def rd(g, s0, s1, b, r0, nr, slot):
            idx = (pl.ds(g, 1), pl.ds(s0, s1 - s0), pl.ds(b, 1), pl.ds(r0, nr))
            return pltpu.make_async_copy(x_hbm.at[idx], buf.at[idx], sems.at[slot])

        def group_copies(i):
            out = []
            for j in range(NC):
                g, b = gb(i * NC + j)
                out += [((g, s0, s1, b, r0, KD), prio)
                        for r0 in range(0, K, KD) for (s0, s1, prio) in PARTS]
            return out

        def tail_copies(cgs):
            out = []
            for cg in cgs:
                for s in range(S):
                    g, b = gb((NG - 1) * NC + jof(cg, s))
                    out.append(((g, s, s + 1, b, 0, K), int(s > 0)))
            return out

        def start(copies, slot):
            for (args, prio) in copies:
                rd(*args, slot).start(priority=prio)

        def wait(copies, slot):
            for (args, _) in copies:
                rd(*args, slot).wait()

        def block_reduce(i, cg):
            sa = ma = None
            for s in range(S):
                g, b = gb(i * NC + jof(cg, s))
                v = buf[g, s, b].astype(F32)
                sa = v if sa is None else sa + v
                ma = v if ma is None else jnp.maximum(ma, v)
            return sa, ma

        def accumulate(i, first=False):
            for cg in range(NC):
                rows = pl.ds(cg * K, K)
                sa, ma = block_reduce(i, cg)
                if first:
                    sum_ref[rows, :] = sa
                    max_ref[rows, :] = ma
                else:
                    sum_ref[rows, :] = sum_ref[rows, :] + sa
                    max_ref[rows, :] = jnp.maximum(max_ref[rows, :], ma)

        start(group_copies(0), 0)
        cw1 = pltpu.make_async_copy(w1t_hbm, w1t_v, sems.at[0])
        cw2 = pltpu.make_async_copy(w2_hbm, w2_v, sems.at[0])
        cw1.start()
        cw2.start()
        for i in range(1, D):
            start(group_copies(i), i)

        wait(group_copies(0), 0)
        cw1.wait()
        cw2.wait()
        start(group_copies(D), 0)
        accumulate(0, first=True)
        jj = jax.lax.broadcasted_iota(jnp.int32, (R, 128), 0)
        ll = jax.lax.broadcasted_iota(jnp.int32, (R, 128), 1)
        sel = jnp.where((ll == jj) | (ll == jj + 64), 1.0, 0.0).astype(BF16)
        dn = (((0,), (0,)), ((), ()))
        w1d_ref[...] = jax.lax.dot_general(w1t_v[...], sel, dn, preferred_element_type=F32)
        w2d_ref[...] = jax.lax.dot_general(w2_v[...], sel, dn, preferred_element_type=F32)

        def body(i, carry):
            slot = jax.lax.rem(i, D)
            wait(group_copies(i), slot)
            start(group_copies(i + D), slot)
            accumulate(i)
            return carry

        nfull = NG - 1
        jax.lax.fori_loop(1, nfull - D, body, 0)

        offs = [sum(TAIL[:i]) for i in range(len(TAIL) + 1)]
        pieces = [tuple(range(offs[i], offs[i + 1])) for i in range(len(TAIL))]
        rest = [(i, None) for i in range(nfull - D, nfull)] + [(NG - 1, pc) for pc in pieces]
        hpart = jnp.zeros((8, 128), F32)
        ready = []
        for k, (i, pc) in enumerate(rest):
            slot = (nfull - D + k) % D
            wait(group_copies(i) if pc is None else tail_copies(pc), slot)
            if k + D < len(rest):
                i2, pc2 = rest[k + D]
                start(group_copies(i2) if pc2 is None else tail_copies(pc2), slot)
            if pc is None:
                accumulate(i)
                continue
            for cg in pc:
                rows = pl.ds(cg * K, K)
                sa, ma = block_reduce(i, cg)
                ready.append((rows, sum_ref[rows, :] + sa, jnp.maximum(max_ref[rows, :], ma)))
            if k == len(rest) - 2:
                continue
            for (rows, tot, mx) in ready:
                gap = jnp.broadcast_to(jnp.sum(tot, axis=1, keepdims=True), (K, 128))
                gap = _rnd(gap * inv_n)
                gmp = jnp.broadcast_to(jnp.max(mx, axis=1, keepdims=True), (K, 128))
                lane = jax.lax.broadcasted_iota(jnp.int32, (K, 128), 1)
                pr = jnp.where(lane < 64, gap, gmp) * w1d_ref[rows, :]
                for r in range(K // 8):
                    hpart = hpart + pr[r * 8:(r + 1) * 8, :]
            ready = []

        osem = sems.at[0]

        def scale_blk(g, s, b, sc):
            buf[g, s, b] = (buf[g, s, b].astype(F32) * sc).astype(BF16)

        def wr(g, s0, s1, b):
            idx = (pl.ds(g, 1), pl.ds(s0, s1 - s0), pl.ds(b, 1))
            pltpu.make_async_copy(buf.at[idx], o_hbm.at[idx], osem).start()

        h = jnp.sum(hpart, axis=0, keepdims=True)
        h = jnp.maximum(_rnd(h), 0.0)
        for cg in range(NC):
            rows = pl.ds(cg * K, K)
            z = jnp.sum(w2d_ref[rows, :] * h, axis=1, keepdims=True)
            z = _rnd(jnp.broadcast_to(z, (K, 128)))
            sc = _rnd(jax.nn.sigmoid(z))
            sc = jnp.concatenate([sc, sc[:, :W - 128]], axis=1)
            scale_ref[rows, :] = sc
            for s in range(S):
                g, b = gb(jof(cg, s))
                scale_blk(g, s, b, sc)
                wr(g, s, s + 1, b)

        def obody(i, carry):
            for j in range(NC):
                g, b = gb(i * NC + j)
                for s in range(S):
                    cg = (j + sh * s) % NC
                    scale_blk(g, s, b, scale_ref[pl.ds(cg * K, K), :])
                wr(g, 0, S, b)
            return carry

        jax.lax.fori_loop(1, NG, obody, 0)
        pltpu.make_async_copy(buf, o_hbm, osem).wait()

    xt = jnp.transpose(x, (0, 1, 3, 2)).reshape(shp)
    o = pl.pallas_call(
        kernel,
        out_shape=jax.ShapeDtypeStruct(shp, x.dtype),
        in_specs=[pl.BlockSpec(memory_space=pl.ANY)] * 3,
        out_specs=pl.BlockSpec(memory_space=pl.ANY),
        scratch_shapes=[
            pltpu.VMEM(shp, x.dtype),
            pltpu.VMEM((R, C), w1.dtype),
            pltpu.VMEM((R, C), w2.dtype),
            pltpu.VMEM((C, 128), F32),
            pltpu.VMEM((C, 128), F32),
            pltpu.VMEM((C, W), F32),
            pltpu.VMEM((C, W), F32),
            pltpu.VMEM((C, W), F32),
            pltpu.SemaphoreType.DMA((D,)),
        ],
        compiler_params=pltpu.CompilerParams(**_COMPILER_PARAMS),
    )(xt, w1.T, w2)
    return jnp.transpose(o.reshape(Bn, H, C, W), (0, 1, 3, 2))
```
